```python
import jax
import jax.numpy as jnp

def _softmax(x, axis=-1):
    return jax.nn.softmax(x, axis=axis)
def _gelu(x):
    return jax.nn.gelu(x, approximate=True)
def _silu(x):
    return jax.nn.silu(x)
def _sigmoid(x):
    return jax.nn.sigmoid(x)
def _layernorm(x, axis=-1, eps=1e-5):
    m = jnp.mean(x, axis=axis, keepdims=True)
    v = jnp.var(x, axis=axis, keepdims=True)
    return (x - m) / jnp.sqrt(v + eps)
def _scatter_add(tgt, idx, src, axis=0):
    return tgt.at[idx].add(src)
def _segment_sum(src, seg, n):
    return jax.ops.segment_sum(src, seg, n)
class _Rng:
    def __init__(self, key):
        self._k = key
    def _next(self):
        self._k, sub = jax.random.split(self._k)
        return sub
    def normal(self, shape):
        return jax.random.normal(self._next(), shape, dtype=jnp.bfloat16)
    def randint(self, lo, hi, shape):
        return jax.random.randint(self._next(), shape, lo, hi, dtype=jnp.int32)
    def uniform(self, shape, lo=0.0, hi=1.0):
        return jax.random.uniform(self._next(), shape, jnp.bfloat16, lo, hi)
    def permutation(self, n):
        return jax.random.permutation(self._next(), n)


kernel_name = 'concat_heads__gqa_block_cached__mha_block_cached__near_ridge'

def setup_inputs():
    _rng = _Rng(jax.random.key(int.from_bytes(__import__("os").urandom(4), "little")))
    _w = (lambda a: (lambda t: t.astype(jnp.bfloat16) if jnp.issubdtype(t.dtype, jnp.floating) else t)(jnp.asarray(a)))
    def _A_setup():
        B, Sq, D = 16, 160, 640
        Hq, Hkv, Sk, Dh = 32, 32, 512, 192
        assert Hq % Hkv == 0, (Hq, Hkv)
        return {
            "x": _w((lambda *s: _rng.normal(s) * 0.05)(B, Sq, D)),
            "k_cache": _w((lambda *s: _rng.normal(s) * 0.05)(B, Hkv, Sk, Dh)),
            "v_cache": _w((lambda *s: _rng.normal(s) * 0.05)(B, Hkv, Sk, Dh)),
            "wq": _w((lambda *s: _rng.normal(s) * 0.05)(D, Hq * Dh) * (D ** -0.5)),
            "wo": _w((lambda *s: _rng.normal(s) * 0.05)(Hq * Dh, D) * ((Hq * Dh) ** -0.5)),
        }
    _A_in = _A_setup()

    def _B_setup():
        B, Sq, D = 16, 160, 640
        H, Sk, Dh = 32, 512, 192
        return {
            "x": _w((lambda *s: _rng.normal(s) * 0.05)(B, Sq, D)),
            "k_cache": _w((lambda *s: _rng.normal(s) * 0.05)(B, H, Sk, Dh)),
            "v_cache": _w((lambda *s: _rng.normal(s) * 0.05)(B, H, Sk, Dh)),
            "wq": _w((lambda *s: _rng.normal(s) * 0.05)(D, H * Dh) * (D ** -0.5)),
            "wo": _w((lambda *s: _rng.normal(s) * 0.05)(H * Dh, D) * ((H * Dh) ** -0.5)),
        }
    _B_in = _B_setup()

    return {
        "A_x": _A_in["x"],
        "A_k_cache": _A_in["k_cache"],
        "A_v_cache": _A_in["v_cache"],
        "A_wq": _A_in["wq"],
        "A_wo": _A_in["wo"],
        "B_x": _B_in["x"],
        "B_k_cache": _B_in["k_cache"],
        "B_v_cache": _B_in["v_cache"],
        "B_wq": _B_in["wq"],
        "B_wo": _B_in["wo"],
    }

def reference(A_x, A_k_cache, A_v_cache, A_wq, A_wo, B_x, B_k_cache, B_v_cache, B_wq, B_wo):
    def _A_ref(x, k_cache, v_cache, wq, wo):
        B, Sq, D = x.shape
        Hq, Dh = 32, 192
        Hkv = k_cache.shape[1]
        rep = Hq // Hkv
        q = (lambda x, *d: x.transpose(*d))((x @ wq).reshape(B, Sq, Hq, Dh), 0, 2, 1, 3)
        k = jnp.repeat(k_cache, rep, axis=1)
        v = jnp.repeat(v_cache, rep, axis=1)
        scores = jnp.einsum("bhqd,bhkd->bhqk", q, k) * (Dh ** -0.5)
        p = _softmax(scores, axis=-1)
        o = jnp.einsum("bhqk,bhkd->bhqd", p, v)
        return (lambda x, *d: x.transpose(*d))(o, 0, 2, 1, 3).reshape(B, Sq, Hq * Dh) @ wo

    def _B_ref(x, k_cache, v_cache, wq, wo):
        B, Sq, D = x.shape
        H, Dh = 32, 192
        q = (lambda x, *d: x.transpose(*d))((x @ wq).reshape(B, Sq, H, Dh), 0, 2, 1, 3)
        scores = jnp.einsum("bhqd,bhkd->bhqk", q, k_cache) * (Dh ** -0.5)
        p = _softmax(scores, axis=-1)
        o = jnp.einsum("bhqk,bhkd->bhqd", p, v_cache)
        return (lambda x, *d: x.transpose(*d))(o, 0, 2, 1, 3).reshape(B, Sq, H * Dh) @ wo

    a = _A_ref(A_x, A_k_cache, A_v_cache, A_wq, A_wo)
    b = _B_ref(B_x, B_k_cache, B_v_cache, B_wq, B_wo)
    return jnp.concatenate([a, b], axis=-1)
```

```python
import functools
import jax
import jax.numpy as jnp
from jax import lax
from jax.experimental import pallas as pl
from jax.experimental.pallas import tpu as pltpu

B, SQ, D, H, SK, DH = 16, 160, 640, 32, 512, 192
LOG2E = 1.4426950408889634
NT = (((1,), (1,)), ((), ()))

def _build(G=4):
    NP = G // 2
    NG = H // G
    c = (DH ** -0.5) * LOG2E

    def kern(xa, ka, va, wqa, woa, xb, kb, vb, wqb, wob, o_ref, xs, acc):
        g = pl.program_id(0)
        b = pl.program_id(1)

        @pl.when(g == 0)
        def _():
            xs[0, b] = xa[0]
            xs[1, b] = xb[0]
            acc[0, b] = jnp.zeros((SQ, D), jnp.float32)
            acc[1, b] = jnp.zeros((SQ, D), jnp.float32)

        lane = lax.broadcasted_iota(jnp.int32, (SQ, 128), 1)
        lo = lane < 64
        for br, (k_ref, v_ref, wq_ref, wo_ref) in enumerate(((ka, va, wqa, woa), (kb, vb, wqb, wob))):
            x = xs[br, b]
            os = []
            for p in range(NP):
                q = jnp.dot(x, wq_ref[:, p*384:(p+1)*384], preferred_element_type=jnp.float32) * c
                t0 = q[:, 0:128].astype(jnp.bfloat16)
                t1 = q[:, 128:256]
                t2 = q[:, 256:384].astype(jnp.bfloat16)
                t1l = jnp.where(lo, t1, 0.0).astype(jnp.bfloat16)
                t1h = jnp.where(lo, 0.0, t1).astype(jnp.bfloat16)
                r0 = p * 384
                s0 = jnp.dot(jnp.concatenate([t0, t1l], 1), k_ref[0, r0:r0+256, :], preferred_element_type=jnp.float32)
                s1 = jnp.dot(jnp.concatenate([t1h, t2], 1), k_ref[0, r0+128:r0+384, :], preferred_element_type=jnp.float32)
                def sm(s):
                    m = jnp.max(s, axis=1, keepdims=True)
                    e = jnp.exp2(s - m)
                    l = jnp.sum(e, axis=1, keepdims=True)
                    return e.astype(jnp.bfloat16), 1.0 / l
                p0, i0 = sm(s0)
                p1, i1 = sm(s1)
                o0 = lax.dot_general(p0, v_ref[0, r0:r0+256, :], NT, preferred_element_type=jnp.float32) * i0
                o1 = lax.dot_general(p1, v_ref[0, r0+128:r0+384, :], NT, preferred_element_type=jnp.float32) * i1
                os += [o0[:, :128].astype(jnp.bfloat16),
                       jnp.where(lo, o0[:, 128:], o1[:, :128]).astype(jnp.bfloat16),
                       o1[:, 128:].astype(jnp.bfloat16)]
            o = jnp.concatenate(os, 1)
            acc[br, b] += jnp.dot(o, wo_ref[...], preferred_element_type=jnp.float32)

        @pl.when(g == NG - 1)
        def _():
            o_ref[0, :, 0:D] = acc[0, b].astype(o_ref.dtype)
            o_ref[0, :, D:2*D] = acc[1, b].astype(o_ref.dtype)

    xspec = pl.BlockSpec((1, SQ, D), lambda g, b: (jnp.where(g == 0, b, B - 1), 0, 0))
    kspec = pl.BlockSpec((1, G * DH, SK), lambda g, b: (b, g, 0))
    wqspec = pl.BlockSpec((D, G * DH), lambda g, b: (0, g))
    wospec = pl.BlockSpec((G * DH, D), lambda g, b: (g, 0))

    @jax.jit
    def fn(A_x, A_k, A_v, A_wq, A_wo, B_x, B_k, B_v, B_wq, B_wo):
        tr = lambda t: jnp.swapaxes(t, 2, 3).reshape(B, H * DH, SK)
        return pl.pallas_call(
            kern,
            grid=(NG, B),
            in_specs=[xspec, kspec, kspec, wqspec, wospec] * 2,
            out_specs=pl.BlockSpec((1, SQ, 2 * D), lambda g, b: (jnp.where(g == NG - 1, b, 0), 0, 0)),
            out_shape=jax.ShapeDtypeStruct((B, SQ, 2 * D), jnp.bfloat16),
            scratch_shapes=[pltpu.VMEM((2, B, SQ, D), jnp.bfloat16), pltpu.VMEM((2, B, SQ, D), jnp.float32)],
            compiler_params=pltpu.CompilerParams(dimension_semantics=("arbitrary", "arbitrary"), vmem_limit_bytes=100 * 1024 * 1024),
            name="attn",
        )(A_x, tr(A_k), tr(A_v), A_wq, A_wo, B_x, tr(B_k), tr(B_v), B_wq, B_wo)
    return fn


_kernel = _build(G=4)


@jax.jit
def pallas_concat_heads__gqa_block_cached__mha_block_cached__near_ridge_kernel(
    A_x, A_k_cache, A_v_cache, A_wq, A_wo, B_x, B_k_cache, B_v_cache, B_wq, B_wo
):
    return _kernel(A_x, A_k_cache, A_v_cache, A_wq, A_wo, B_x, B_k_cache, B_v_cache, B_wq, B_wo)
```

```python
import contextlib
import functools
import jax
import jax.numpy as jnp
from jax import lax
from jax.experimental import pallas as pl
from jax.experimental.pallas import tpu as pltpu

B, SQ, D, H, SK, DH = 16, 160, 640, 32, 512, 192
LOG2E = 1.4426950408889634
NT = (((1,), (1,)), ((), ()))
F32, BF16 = jnp.float32, jnp.bfloat16
PW = 2 * DH

def div(a, n):
    if isinstance(a, int):
        return a // n
    assert n & (n - 1) == 0
    return lax.shift_right_logical(a, n.bit_length() - 1)


def mod(a, n):
    if isinstance(a, int):
        return a % n
    assert n & (n - 1) == 0
    return lax.bitwise_and(a, n - 1)


def _build(NB=2, NP=4, order='a', flags=None, only=None, NSLOT=2, PB=4, PP=1, scopes=False, nobc=True, startpos=0, tailq=0):
    GW = NP * PW
    NG = H // (2 * NP)
    NBG = B // NB
    NIT = NG * NBG
    c = (DH ** -0.5) * LOG2E
    sus = [(br, j) for j in range(NB) for br in range(2)]
    NS = len(sus)
    NPB, NPP = B // PB, NP // PP
    scope = jax.named_scope if scopes else (lambda n: contextlib.nullcontext())

    def kern(xa, ka, va, wqa, woa, xb, kb, vb, wqb, wob, out,
             xs, acc, qs, kbuf, vbuf, wq, wo, obuf, kvsem, wsem, xsem, psem, osem):
        X, K, V, WQ, WO = (xa, xb), (ka, kb), (va, vb), (wqa, wqb), (woa, wob)

        def kv_copies(it, slot):
            g = div(it, NBG)
            b0 = (mod(it, NBG)) * NB
            cps = []
            for br in range(2):
                cps.append(pltpu.make_async_copy(K[br].at[pl.ds(b0, NB), pl.ds(g * GW, GW), :], kbuf.at[slot, br], kvsem.at[slot, 0, br]))
                cps.append(pltpu.make_async_copy(V[br].at[pl.ds(b0, NB), pl.ds(g * GW, GW), :], vbuf.at[slot, br], kvsem.at[slot, 1, br]))
            return cps

        def wq_copy(br, g):
            off = g * GW if isinstance(g, int) else pl.multiple_of(g * GW, 128)
            return pltpu.make_async_copy(WQ[br].at[:, pl.ds(off, GW)], wq.at[mod(g, 2), br], wsem.at[mod(g, 2), 0, br])

        def wq0_copy(br, h):
            w = PP * PW
            off = h * w if isinstance(h, int) else pl.multiple_of(h * w, 128)
            return pltpu.make_async_copy(WQ[br if isinstance(br, int) else 0].at[:, pl.ds(off, w)], wq.at[0, br, :, pl.ds(off, w)], psem.at[br, h])

        def wo_copy(br, g):
            off = g * GW if isinstance(g, int) else pl.multiple_of(g * GW, 128)
            return pltpu.make_async_copy(WO[br].at[pl.ds(off, GW), :], wo.at[mod(g, 2), br], wsem.at[mod(g, 2), 1, br])

        def x_copy(br, i):
            return pltpu.make_async_copy(X[br if isinstance(br, int) else 0].at[pl.ds(i * PB, PB)], xs.at[br, pl.ds(i * PB, PB)], xsem.at[br, i])

        def o_copy(b):
            return pltpu.make_async_copy(obuf.at[b], out.at[b], osem.at[b])

        lo = lax.broadcasted_iota(jnp.int32, (SQ, 128), 1) < 64

        def qproj(br, b, ws, p):
            off = p * PW if isinstance(p, int) else pl.multiple_of(p * PW, 128)
            q = jnp.dot(xs[br, b], wq[ws, br, :, pl.ds(off, PW)], preferred_element_type=F32) * c
            t1 = q[:, 128:256]
            qr = qs.at[br, b, p]
            qr[:, 0:128] = q[:, 0:128].astype(BF16)
            qr[:, 128:256] = jnp.where(lo, t1, 0.0).astype(BF16)
            qr[:, 256:384] = jnp.where(lo, 0.0, t1).astype(BF16)
            qr[:, 384:512] = q[:, 256:384].astype(BF16)

        def step(it, last):
            g = div(it, NBG)
            b0 = (mod(it, NBG)) * NB
            slot = mod(it, NSLOT)
            ws = mod(g, 2)

            def prefetch():
                nxt = it + NSLOT - 1
                if last:
                    nxt = jnp.minimum(nxt, NIT - 1)
                for cp in kv_copies(nxt, mod(it + NSLOT - 1, NSLOT)):
                    cp.start()

            def qk(i, p):
                br, j = sus[i]
                qr = qs.at[br, b0 + j, p]
                kr = kbuf.at[slot, br, j]
                s0 = jnp.dot(qr[:, 0:256], kr[p * PW:p * PW + 256, :], preferred_element_type=F32)
                s1 = jnp.dot(qr[:, 256:512], kr[p * PW + 128:p * PW + 384, :], preferred_element_type=F32)
                return s0, s1

            def sm(s):
                m = jnp.max(s, axis=1, keepdims=True)
                e = jnp.exp2(s - m)
                l = jnp.sum(e, axis=1, keepdims=True)
                return e.astype(BF16), pltpu.reciprocal(l, full_range=False)

            def pvf(i, p, s):
                br, j = sus[i]
                p0, i0 = sm(s[0])
                p1, i1 = sm(s[1])
                vr = vbuf.at[slot, br, j]
                r = p * PW
                dnt = lambda a, b: lax.dot_general(a, b, NT, preferred_element_type=F32)
                o0a = dnt(p0, vr[r:r + 128, :]) * i0
                o0bt = dnt(vr[r + 128:r + 192, :], p0[0:128])
                o1a = dnt(p1, vr[r + 256:r + 384, :]) * i1
                o1bt = dnt(vr[r + 192:r + 256, :], p1[0:128])
                orem = dnt(jnp.concatenate([p0[128:160], p1[128:160]], 0), vr[r + 128:r + 256, :])
                obm = jnp.concatenate([o0bt, o1bt], 0).T
                obr = jnp.where(lo[0:32], orem[0:32], orem[32:64])
                ob = jnp.concatenate([obm, obr], 0) * jnp.where(lo, i0, i1)
                return [o0a.astype(BF16), ob.astype(BF16), o1a.astype(BF16)]

            def oproj(i, o, n0=0, n1=D):
                br, j = sus[i]
                o = jnp.concatenate(o, 1)
                r = acc[br, b0 + j, :, n0:n1] + jnp.dot(o, wo[ws, br, :, n0:n1], preferred_element_type=F32)
                if last:
                    obuf[b0 + j, :, br * D + n0:br * D + n1] = r.astype(BF16)
                    if br == 1 and n1 == D:
                        o_copy(b0 + j).start()
                else:
                    acc[br, b0 + j, :, n0:n1] = r

            def qnext(i, p):
                if not last:
                    br, j = sus[i]
                    qproj(br, b0 + j, 1 - ws, p)

            cuts = {1: [0, D], 2: [0, 256, D], 4: [0, 128, 256, 384, D]}[NP]
            prs = [(i, p) for i in range(NS) for p in range(NP)]
            o_prev, o = None, []
            if startpos < 0:
                prefetch()
            for n, (i, p) in enumerate(prs):
                s = qk(i, p)
                if n == startpos:
                    prefetch()
                if n < len(prs) - tailq:
                    qnext(i, p)
                if o_prev is not None:
                    oproj(i - 1, o_prev, cuts[p], cuts[p + 1])
                o += pvf(i, p, s)
                if p == NP - 1:
                    o_prev, o = o, []
            for n in range(len(prs) - tailq, len(prs)):
                qnext(*prs[n])
            oproj(NS - 1, o_prev)

        def zero(lo_b, hi_b):
            def z(b, _):
                for br in range(2):
                    acc[br, b] = jnp.zeros((SQ, D), F32)
            lax.fori_loop(lo_b, hi_b, z, None)

        wq0_copy(0, 0).start()
        x_copy(0, 0).start()
        zero(0, 3)
        for i in range(1, NPB):
            x_copy(0, i).start()
        zero(3, 6)
        for h in range(1, NPP):
            wq0_copy(0, h).start()
        wq0_copy(1, 0).start()
        zero(6, 9)
        for i in range(NPB):
            x_copy(1, i).start()
        zero(9, 12)
        for h in range(1, NPP):
            wq0_copy(1, h).start()
        zero(12, B)
        for cp in kv_copies(0, 0):
            cp.start()
        for br in range(2):
            wq_copy(br, 1).start()
            wo_copy(br, 0).start()

        def pro(t, _):
            br = div(t, NPP * NPB)
            h = mod(div(t, NPB), NPP)
            i = mod(t, NPB)

            @pl.when(i == 0)
            def _():
                wq0_copy(br, h).wait()

            @pl.when(h == 0)
            def _():
                x_copy(br, i).wait()

            for j in range(PB):
                for p in range(PP):
                    qproj(br, i * PB + j, 0, h * PP + p)
        if only is None:
            with scope("pro"):
                lax.fori_loop(0, 2 * NPP * NPB, pro, None)

        def head(it, last):
            g = div(it, NBG)
            bg = mod(it, NBG)
            if last:
                @pl.when(bg == 0)
                def _():
                    for br in range(2):
                        wo_copy(br, g).wait()
            else:
                @pl.when(bg == 0)
                def _():
                    for br in range(2):
                        wq_copy(br, g + 1).wait()
                        wo_copy(br, g).wait()

                for br in range(2):
                    @pl.when(bg == br * (NBG // 4))
                    def _():
                        wo_copy(br, g + 1).start()

                    @pl.when(jnp.logical_and(bg == (2 + br) * (NBG // 4), g + 2 < NG))
                    def _():
                        wq_copy(br, g + 2).start()
            for cp in kv_copies(it, mod(it, NSLOT)):
                cp.wait()

        def body(it, _):
            with scope("head"):
                head(it, False)
            with scope("step"):
                step(it, False)

        def body_last(it, _):
            with scope("headl"):
                head(it, True)
            with scope("stepl"):
                step(it, True)

        if only in (None, 'main'):
            lax.fori_loop(0, NIT - NBG, body, None)
        if only in (None, 'last'):
            lax.fori_loop(NIT - NBG, NIT, body_last, None)
        with scope("tail"):
            for i in range(NSLOT - 1):
                for cp in kv_copies(NIT - 1, (NIT + i) % NSLOT):
                    cp.wait()
            for b in range(B):
                o_copy(b).wait()

    @jax.jit
    def fn(A_x, A_k, A_v, A_wq, A_wo, B_x, B_k, B_v, B_wq, B_wo):
        tr = lambda t: jnp.swapaxes(t, 2, 3).reshape(B, H * DH, SK)
        return pl.pallas_call(
            kern,
            in_specs=[pl.BlockSpec(memory_space=pl.ANY)] * 10,
            out_specs=pl.BlockSpec(memory_space=pl.ANY),
            out_shape=jax.ShapeDtypeStruct((B, SQ, 2 * D), BF16),
            scratch_shapes=[
                pltpu.VMEM((2, B, SQ, D), BF16),
                pltpu.VMEM((2, B, SQ, D), F32),
                pltpu.VMEM((2, B, NP, SQ, 512), BF16),
                pltpu.VMEM((NSLOT, 2, NB, GW, SK), BF16),
                pltpu.VMEM((NSLOT, 2, NB, GW, SK), BF16),
                pltpu.VMEM((2, 2, D, GW), BF16),
                pltpu.VMEM((2, 2, GW, D), BF16),
                pltpu.VMEM((B, SQ, 2 * D), BF16),
                pltpu.SemaphoreType.DMA((NSLOT, 2, 2)),
                pltpu.SemaphoreType.DMA((2, 2, 2)),
                pltpu.SemaphoreType.DMA((2, NPB)),
                pltpu.SemaphoreType.DMA((2, NPP)),
                pltpu.SemaphoreType.DMA((B,)),
            ],
            compiler_params=pltpu.CompilerParams(vmem_limit_bytes=124 * 1024 * 1024, flags=flags, disable_bounds_checks=nobc),
            name="attn",
        )(A_x, tr(A_k), tr(A_v), A_wq, A_wo, B_x, tr(B_k), tr(B_v), B_wq, B_wo)
    return fn


_kernel = _build()


@jax.jit
def pallas_concat_heads__gqa_block_cached__mha_block_cached__near_ridge_kernel(
    A_x, A_k_cache, A_v_cache, A_wq, A_wo, B_x, B_k_cache, B_v_cache, B_wq, B_wo
):
    return _kernel(A_x, A_k_cache, A_v_cache, A_wq, A_wo, B_x, B_k_cache, B_v_cache, B_wq, B_wo)
```

```python
import contextlib

import jax
import jax.numpy as jnp
from jax import lax
from jax.experimental import pallas as pl
from jax.experimental.pallas import tpu as pltpu

B, SQ, D, H, SK, DH = 16, 160, 640, 32, 512, 192
LOG2E = 1.4426950408889634
F32, BF16 = jnp.float32, jnp.bfloat16
PW = 2 * DH


def div(a, n):
    if isinstance(a, int):
        return a // n
    assert n & (n - 1) == 0
    return lax.shift_right_logical(a, n.bit_length() - 1)


def mod(a, n):
    if isinstance(a, int):
        return a % n
    assert n & (n - 1) == 0
    return lax.bitwise_and(a, n - 1)


def lanes(k, w):
    return pl.ds(k * w if isinstance(k, int) else pl.multiple_of(k * w, 128), w)


def dot_nn(a, b):
    return jnp.dot(a, b, preferred_element_type=F32)


def dot_nt(a, b):
    return lax.dot_general(a, b, (((1,), (1,)), ((), ())), preferred_element_type=F32)


def _build(NB=2, NP=4, PP=2, LEAD=5, order='koqv', pvord='acbde', only=None, scopes=False, flags=None,
         startpos=0, wpos=1, tailsplit=1):
    GW = NP * PW
    NG = H // (2 * NP)
    NBG = B // NB
    NIT = NG * NBG
    NPP = NP // PP
    c = (DH ** -0.5) * LOG2E
    sus = [(br, j) for j in range(NB) for br in range(2)]
    prs = [(i, p) for i in range(len(sus)) for p in range(NP)]
    cuts = {1: [0, D], 2: [0, 256, D], 4: [0, 128, 256, 384, D]}[NP]
    scope = jax.named_scope if scopes else (lambda n: contextlib.nullcontext())

    def kern(xa, ka, va, wqa, woa, xb, kb, vb, wqb, wob, out,
             xs, acc, qs, kv, wq, wo, obuf, kvsem, wqsem, wosem, xsem, psem, osem):
        X, K, V, WQ, WO = (xa, xb), (ka, kb), (va, vb), (wqa, wqb), (woa, wob)

        def kv_start(it):
            slot = mod(it, 2)
            b0 = mod(it, NBG) * NB
            rows = pl.ds(div(it, NBG) * GW, GW)
            for br in range(2):
                for t, src in enumerate((K, V)):
                    pltpu.make_async_copy(src[br].at[pl.ds(b0, NB), rows, :], kv.at[slot, br, t], kvsem.at[slot]).start()

        def whole(buf, sem, slot):
            return pltpu.make_async_copy(buf.at[slot], buf.at[slot], sem.at[slot])

        def wq_copy(br, g):
            return pltpu.make_async_copy(WQ[br].at[:, lanes(g, GW)], wq.at[mod(g, 2), br], wqsem.at[mod(g, 2)])

        def wo_copy(br, g):
            return pltpu.make_async_copy(WO[br].at[lanes(g, GW), :], wo.at[mod(g, 2), br], wosem.at[mod(g, 2)])

        def wq0_copy(br, h):
            src = WQ[br] if isinstance(br, int) else WQ[0]
            return pltpu.make_async_copy(src.at[:, lanes(h, PP * PW)], wq.at[0, br, :, lanes(h, PP * PW)], psem.at[br, h])

        def x_copy(br, i):
            src = X[br] if isinstance(br, int) else X[0]
            return pltpu.make_async_copy(src.at[pl.ds(i * NB, NB)], xs.at[br, pl.ds(i * NB, NB)], xsem.at[br, i])

        def o_copy(b, c0, c1):
            return pltpu.make_async_copy(obuf.at[b, :, c0:c1], out.at[b, :, c0:c1], osem)

        lo = lax.broadcasted_iota(jnp.int32, (SQ, 128), 1) < 64

        def qproj(br, b, ws, p):
            q = dot_nn(xs[br, b], wq[ws, br, :, lanes(p, PW)]) * c
            mid = q[:, 128:256]
            qr = qs.at[br, b, p]
            qr[0] = q[:, 0:128].astype(BF16)
            qr[1] = jnp.where(lo, mid, 0.0).astype(BF16)
            qr[2] = jnp.where(lo, 0.0, mid).astype(BF16)
            qr[3] = q[:, 256:384].astype(BF16)

        def softmax_parts(s):
            e = jnp.exp2(s - jnp.max(s, axis=1, keepdims=True))
            return e, pltpu.reciprocal(jnp.sum(e, axis=1, keepdims=True), full_range=False)

        def step(it, last):
            g = div(it, NBG)
            bg = mod(it, NBG)
            b0 = bg * NB
            slot = mod(it, 2)
            gq = div(it + LEAD, NBG)
            bgq = mod(it + LEAD, NBG)

            with scope("headl" if last else "head"):
                @pl.when(bg == 0)
                def _():
                    whole(wo, wosem, mod(g, 2)).wait()

                if not last:
                    @pl.when(bgq == 0)
                    def _():
                        whole(wq, wqsem, mod(gq, 2)).wait()

                    @pl.when(gq == 0)
                    def _():
                        for br in range(2):
                            x_copy(br, bgq).wait()

                whole(kv, kvsem, slot).wait()

            def prefetch_kv():
                if last:
                    pl.when(it + 1 < NIT)(lambda: kv_start(it + 1))
                else:
                    kv_start(it + 1)

            def prefetch_w():
                if last:
                    return
                for br in range(2):
                    pl.when(jnp.logical_and(bg == 1 + br, g + 1 < NG))(wo_copy(br, jnp.minimum(g + 1, NG - 1)).start)
                    pl.when(jnp.logical_and(bgq == NBG - 3 + br, gq + 1 < NG))(wq_copy(br, jnp.minimum(gq + 1, NG - 1)).start)

            def qk(i, p):
                br, j = sus[i]
                qr = qs.at[br, b0 + j, p]
                kr = kv.at[slot, br, 0, j]
                r = p * PW
                s0 = dot_nn(jnp.concatenate([qr[0], qr[1]], 1), kr[r:r + 256, :])
                s1 = dot_nn(jnp.concatenate([qr[2], qr[3]], 1), kr[r + 128:r + 384, :])
                return s0, s1

            def pv(i, p, s):
                br, j = sus[i]
                e0, r0 = softmax_parts(s[0])
                e1, r1 = softmax_parts(s[1])
                vr = kv.at[slot, br, 1, j]
                r = p * PW
                res = {}
                for ch in pvord:
                    if ch == 'a': res[ch] = dot_nt(e0.astype(BF16), vr[r:r + 128, :]) * r0
                    if ch == 'b': res[ch] = dot_nt(vr[r + 128:r + 192, :], e0[0:128].astype(BF16))
                    if ch == 'c': res[ch] = dot_nt(e1.astype(BF16), vr[r + 256:r + 384, :]) * r1
                    if ch == 'd': res[ch] = dot_nt(vr[r + 192:r + 256, :], e1[0:128].astype(BF16))
                    if ch == 'e': res[ch] = dot_nt(jnp.concatenate([e0[128:], e1[128:]], 0).astype(BF16), vr[r + 128:r + 256, :])
                o0, o0t, o1, o1t, rem = (res[ch] for ch in 'abcde')
                top = jnp.concatenate([o0t, o1t], 0).T
                bot = jnp.where(lo[0:32], rem[0:32], rem[32:64])
                mid = jnp.concatenate([top, bot], 0) * jnp.where(lo, r0, r1)
                return [o0, mid, o1]

            def oproj(i, o, n0, n1, dma):
                br, j = sus[i]
                o = jnp.concatenate(o, 1).astype(BF16)
                res = acc[br, b0 + j, :, n0:n1] + dot_nn(o, wo[mod(g, 2), br, :, n0:n1])
                if not last:
                    acc[br, b0 + j, :, n0:n1] = res
                if last or LEAD < NBG:
                    obuf[b0 + j, :, br * D + n0:br * D + n1] = res.astype(BF16)
                    if dma is not None:
                        cp = o_copy(b0 + j, br * D + dma, br * D + n1)
                        if last:
                            cp.start()
                        else:
                            pl.when(g == NG - 1)(cp.start)

            with scope("stepl" if last else "step"):
                o_prev, o = None, []
                for n, (i, p) in enumerate(prs):
                    for ch in order:
                        if ch == 'k':
                            s = qk(i, p)
                            if n == startpos:
                                prefetch_kv()
                            if n == wpos:
                                prefetch_w()
                        elif ch == 'o' and o_prev is not None:
                            oproj(i - 1, o_prev, cuts[p], cuts[p + 1], 0 if p == NP - 1 else None)
                        elif ch == 'q' and not last:
                            br, j = sus[i]
                            qproj(br, bgq * NB + j, mod(gq, 2), p)
                        elif ch == 'v':
                            o += pv(i, p, s)
                    if p == NP - 1:
                        o_prev, o = o, []
                tc = {1: [0, D], 2: [0, 512, D], 3: [0, 256, 512, D]}[tailsplit if last else 1]
                for n0, n1 in zip(tc[:-1], tc[1:]):
                    oproj(len(sus) - 1, o_prev, n0, n1, n0)

        def zero(b_lo, b_hi):
            def z(b, _):
                for br in range(2):
                    acc[br, b] = jnp.zeros((SQ, D), F32)
            lax.fori_loop(b_lo, b_hi, z, None)

        wq0_copy(0, 0).start()
        x_copy(0, 0).start()
        zero(0, 3)
        for h in range(1, NPP):
            wq0_copy(0, h).start()
        zero(3, 6)
        wq0_copy(1, 0).start()
        x_copy(1, 0).start()
        zero(6, 9)
        for h in range(1, NPP):
            wq0_copy(1, h).start()
        zero(9, 11)
        for i in range(1, min(LEAD + 1, NBG)):
            for br in range(2):
                x_copy(br, i).start()
        zero(11, 13)
        kv_start(0)
        for br in range(2):
            wo_copy(br, 0).start()
            if LEAD >= NBG - 2:
                wq_copy(br, 1).start()
        zero(13, B)
        for i in range(LEAD + 1, NBG):
            for br in range(2):
                x_copy(br, i).start()

        def pro(t, _):
            i = div(t, 2 * NPP)
            br = mod(div(t, NPP), 2)
            h = mod(t, NPP)
            pl.when(i == 0)(wq0_copy(br, h).wait)
            pl.when(h == 0)(x_copy(br, i).wait)
            for j in range(NB):
                for p in range(PP):
                    qproj(br, i * NB + j, 0, h * PP + p)

        if only is None:
            with scope("pro"):
                lax.fori_loop(0, 2 * NPP * LEAD, pro, None)
        if only in (None, 'main'):
            lax.fori_loop(0, NIT - LEAD, lambda it, _: step(it, False), None)
        if only in (None, 'last'):
            lax.fori_loop(NIT - LEAD, NIT, lambda it, _: step(it, True), None)
        with scope("tail"):
            pltpu.make_async_copy(obuf, out, osem).wait()

    @jax.jit
    def fn(A_x, A_k, A_v, A_wq, A_wo, B_x, B_k, B_v, B_wq, B_wo):
        tr = lambda t: jnp.swapaxes(t, 2, 3).reshape(B, H * DH, SK)
        return pl.pallas_call(
            kern,
            in_specs=[pl.BlockSpec(memory_space=pl.ANY)] * 10,
            out_specs=pl.BlockSpec(memory_space=pl.ANY),
            out_shape=jax.ShapeDtypeStruct((B, SQ, 2 * D), BF16),
            scratch_shapes=[
                pltpu.VMEM((2, B, SQ, D), BF16),
                pltpu.VMEM((2, B, SQ, D), F32),
                pltpu.VMEM((2, B, NP, 4, SQ, 128), BF16),
                pltpu.VMEM((2, 2, 2, NB, GW, SK), BF16),
                pltpu.VMEM((2, 2, D, GW), BF16),
                pltpu.VMEM((2, 2, GW, D), BF16),
                pltpu.VMEM((B, SQ, 2 * D), BF16),
                pltpu.SemaphoreType.DMA((2,)),
                pltpu.SemaphoreType.DMA((2,)),
                pltpu.SemaphoreType.DMA((2,)),
                pltpu.SemaphoreType.DMA((2, NBG)),
                pltpu.SemaphoreType.DMA((2, NPP)),
                pltpu.SemaphoreType.DMA(()),
            ],
            compiler_params=pltpu.CompilerParams(vmem_limit_bytes=120 * 1024 * 1024, flags=flags, disable_bounds_checks=True),
            name="attn",
        )(A_x, tr(A_k), tr(A_v), A_wq, A_wo, B_x, tr(B_k), tr(B_v), B_wq, B_wo)
    return fn


_kernel = _build(tailsplit=2)


@jax.jit
def pallas_concat_heads__gqa_block_cached__mha_block_cached__near_ridge_kernel(
    A_x, A_k_cache, A_v_cache, A_wq, A_wo, B_x, B_k_cache, B_v_cache, B_wq, B_wo
):
    return _kernel(A_x, A_k_cache, A_v_cache, A_wq, A_wo, B_x, B_k_cache, B_v_cache, B_wq, B_wo)
```

```python
import jax
import jax.numpy as jnp
from jax import lax
from jax.experimental import pallas as pl
from jax.experimental.pallas import tpu as pltpu

B, SQ, D, H, SK, DH = 16, 160, 640, 32, 512, 192
F32, BF16 = jnp.float32, jnp.bfloat16

PW = 2 * DH
NB = 2
NP = 4
PP = 2
LEAD = 5
GW = NP * PW
NG = H // (2 * NP)
NBG = B // NB
NIT = NG * NBG
NPP = NP // PP
QSCALE = (DH**-0.5) * 1.4426950408889634
OCUTS = (0, 128, 256, 384, D)


def _div(a, n):
    return a // n if isinstance(a, int) else lax.shift_right_logical(a, n.bit_length() - 1)


def _mod(a, n):
    return a % n if isinstance(a, int) else lax.bitwise_and(a, n - 1)


def _block(k, w):
    return pl.ds(k * w if isinstance(k, int) else pl.multiple_of(k * w, 128), w)


def _dot(a, b):
    return jnp.dot(a, b, preferred_element_type=F32)


def _dot_nt(a, b):
    return lax.dot_general(a, b, (((1,), (1,)), ((), ())), preferred_element_type=F32)


def _wait(dst, sem):
    pltpu.make_async_copy(dst, dst, sem).wait()


def _softmax_parts(s):
    e = jnp.exp2(s - jnp.max(s, axis=1, keepdims=True))
    return e, pltpu.reciprocal(jnp.sum(e, axis=1, keepdims=True), full_range=False)


def _kernel(xa, ka, va, wqa, woa, xb, kb, vb, wqb, wob, out,
            xs, acc, qs, kv, wq, wo, obuf, kvsem, wqsem, wosem, xsem, psem, osem):
    x_hbm, k_hbm, v_hbm = (xa, xb), (ka, kb), (va, vb)
    wq_hbm, wo_hbm = (wqa, wqb), (woa, wob)
    lo = lax.broadcasted_iota(jnp.int32, (SQ, 128), 1) < 64

    def kv_start(it):
        slot = _mod(it, 2)
        batches = pl.ds(_mod(it, NBG) * NB, NB)
        rows = pl.ds(_div(it, NBG) * GW, GW)
        for br in range(2):
            for t, src in enumerate((k_hbm, v_hbm)):
                pltpu.make_async_copy(src[br].at[batches, rows, :], kv.at[slot, br, t], kvsem.at[slot]).start()

    def wq_start(br, g):
        pltpu.make_async_copy(wq_hbm[br].at[:, _block(g, GW)], wq.at[_mod(g, 2), br], wqsem.at[_mod(g, 2)]).start()

    def wo_start(br, g):
        pltpu.make_async_copy(wo_hbm[br].at[_block(g, GW), :], wo.at[_mod(g, 2), br], wosem.at[_mod(g, 2)]).start()

    def wq0_piece(br, h):
        return wq.at[0, br, :, _block(h, PP * PW)]

    def wq0_start(br, h):
        pltpu.make_async_copy(wq_hbm[br].at[:, _block(h, PP * PW)], wq0_piece(br, h), psem.at[br, h]).start()

    def x_piece(br, i):
        return xs.at[br, pl.ds(i * NB, NB)]

    def x_start(br, i):
        pltpu.make_async_copy(x_hbm[br].at[pl.ds(i * NB, NB)], x_piece(br, i), xsem.at[br, i]).start()

    def qproj(br, b, ws, p):
        q = _dot(xs[br, b], wq[ws, br, :, _block(p, PW)]) * QSCALE
        mid = q[:, 128:256]
        qr = qs.at[br, b, p]
        qr[0] = q[:, 0:128].astype(BF16)
        qr[1] = jnp.where(lo, mid, 0.0).astype(BF16)
        qr[2] = jnp.where(lo, 0.0, mid).astype(BF16)
        qr[3] = q[:, 256:384].astype(BF16)

    def step(it, last):
        g, bg = _div(it, NBG), _mod(it, NBG)
        gq, bgq = _div(it + LEAD, NBG), _mod(it + LEAD, NBG)
        b0 = bg * NB
        slot = _mod(it, 2)

        pl.when(bg == 0)(lambda: _wait(wo.at[_mod(g, 2)], wosem.at[_mod(g, 2)]))
        if not last:
            pl.when(bgq == 0)(lambda: _wait(wq.at[_mod(gq, 2)], wqsem.at[_mod(gq, 2)]))

            @pl.when(gq == 0)
            def _():
                for br in range(2):
                    _wait(x_piece(br, bgq), xsem.at[br, bgq])

        _wait(kv.at[slot], kvsem.at[slot])

        def prefetch_kv():
            if last:
                pl.when(it + 1 < NIT)(lambda: kv_start(it + 1))
            else:
                kv_start(it + 1)

        def prefetch_weights():
            for br in range(2):
                pl.when(jnp.logical_and(bg == 1 + br, g + 1 < NG))(lambda: wo_start(br, g + 1))
                pl.when(jnp.logical_and(bgq == LEAD + br, gq + 1 < NG))(lambda: wq_start(br, gq + 1))

        def scores(br, j, p):
            qr = qs.at[br, b0 + j, p]
            kr = kv.at[slot, br, 0, j]
            r = p * PW
            s0 = _dot(jnp.concatenate([qr[0], qr[1]], 1), kr[r:r + 256, :])
            s1 = _dot(jnp.concatenate([qr[2], qr[3]], 1), kr[r + 128:r + 384, :])
            return s0, s1

        def attend(br, j, p, s0, s1):
            e0, r0 = _softmax_parts(s0)
            e1, r1 = _softmax_parts(s1)
            vr = kv.at[slot, br, 1, j]
            r = p * PW
            o0 = _dot_nt(e0.astype(BF16), vr[r:r + 128, :]) * r0
            o1 = _dot_nt(e1.astype(BF16), vr[r + 256:r + 384, :]) * r1
            o0t = _dot_nt(vr[r + 128:r + 192, :], e0[0:128].astype(BF16))
            o1t = _dot_nt(vr[r + 192:r + 256, :], e1[0:128].astype(BF16))
            rem = _dot_nt(jnp.concatenate([e0[128:], e1[128:]], 0).astype(BF16), vr[r + 128:r + 256, :])
            top = jnp.concatenate([o0t, o1t], 0).T
            bot = jnp.where(lo[0:32], rem[0:32], rem[32:64])
            mid = jnp.concatenate([top, bot], 0) * jnp.where(lo, r0, r1)
            return [o0, mid, o1]

        def oproj(br, j, o, n0, n1, flush_from=None):
            o = jnp.concatenate(o, 1).astype(BF16)
            res = acc[br, b0 + j, :, n0:n1] + _dot(o, wo[_mod(g, 2), br, :, n0:n1])
            if not last:
                acc[br, b0 + j, :, n0:n1] = res
            obuf[b0 + j, :, br * D + n0:br * D + n1] = res.astype(BF16)
            if flush_from is not None:
                cols = slice(br * D + flush_from, br * D + n1)
                copy = pltpu.make_async_copy(obuf.at[b0 + j, :, cols], out.at[b0 + j, :, cols], osem)
                if last:
                    copy.start()
                else:
                    pl.when(g == NG - 1)(copy.start)

        prev = None
        for n, (j, br) in enumerate((j, br) for j in range(NB) for br in range(2)):
            o = []
            for p in range(NP):
                s0, s1 = scores(br, j, p)
                if n == 0 and p == 0:
                    prefetch_kv()
                if n == 0 and p == 1 and not last:
                    prefetch_weights()
                if prev is not None:
                    oproj(*prev, OCUTS[p], OCUTS[p + 1], 0 if p == NP - 1 else None)
                if not last:
                    qproj(br, bgq * NB + j, _mod(gq, 2), p)
                o += attend(br, j, p, s0, s1)
            prev = (br, j, o)
        cuts = (0, 512, D) if last else (0, D)
        for n0, n1 in zip(cuts[:-1], cuts[1:]):
            oproj(*prev, n0, n1, n0)

    def zero(b_lo, b_hi):
        def body(b, _):
            for br in range(2):
                acc[br, b] = jnp.zeros((SQ, D), F32)

        lax.fori_loop(b_lo, b_hi, body, None)

    wq0_start(0, 0)
    x_start(0, 0)
    zero(0, 3)
    for h in range(1, NPP):
        wq0_start(0, h)
    zero(3, 6)
    wq0_start(1, 0)
    x_start(1, 0)
    zero(6, 9)
    for h in range(1, NPP):
        wq0_start(1, h)
    zero(9, 11)
    for i in range(1, LEAD + 1):
        for br in range(2):
            x_start(br, i)
    zero(11, 13)
    kv_start(0)
    for br in range(2):
        wo_start(br, 0)
    zero(13, B)
    for i in range(LEAD + 1, NBG):
        for br in range(2):
            x_start(br, i)

    def prologue(t, _):
        i, br, h = _div(t, 2 * NPP), _mod(_div(t, NPP), 2), _mod(t, NPP)
        pl.when(i == 0)(lambda: _wait(wq0_piece(br, h), psem.at[br, h]))
        pl.when(h == 0)(lambda: _wait(x_piece(br, i), xsem.at[br, i]))
        for j in range(NB):
            for p in range(PP):
                qproj(br, i * NB + j, 0, h * PP + p)

    lax.fori_loop(0, 2 * NPP * LEAD, prologue, None)
    lax.fori_loop(0, NIT - LEAD, lambda it, _: step(it, False), None)
    lax.fori_loop(NIT - LEAD, NIT, lambda it, _: step(it, True), None)
    pltpu.make_async_copy(obuf, out, osem).wait()


@jax.jit
def pallas_concat_heads__gqa_block_cached__mha_block_cached__near_ridge_kernel(
    A_x: jax.Array,
    A_k_cache: jax.Array,
    A_v_cache: jax.Array,
    A_wq: jax.Array,
    A_wo: jax.Array,
    B_x: jax.Array,
    B_k_cache: jax.Array,
    B_v_cache: jax.Array,
    B_wq: jax.Array,
    B_wo: jax.Array,
):
    assert A_x.shape == B_x.shape == (B, SQ, D)
    assert A_k_cache.shape == A_v_cache.shape == B_k_cache.shape == B_v_cache.shape == (B, H, SK, DH)

    def dims_major(t):
        return jnp.swapaxes(t, 2, 3).reshape(B, H * DH, SK)

    return pl.pallas_call(
        _kernel,
        in_specs=[pl.BlockSpec(memory_space=pl.ANY)] * 10,
        out_specs=pl.BlockSpec(memory_space=pl.ANY),
        out_shape=jax.ShapeDtypeStruct((B, SQ, 2 * D), BF16),
        scratch_shapes=[
            pltpu.VMEM((2, B, SQ, D), BF16),
            pltpu.VMEM((2, B, SQ, D), F32),
            pltpu.VMEM((2, B, NP, 4, SQ, 128), BF16),
            pltpu.VMEM((2, 2, 2, NB, GW, SK), BF16),
            pltpu.VMEM((2, 2, D, GW), BF16),
            pltpu.VMEM((2, 2, GW, D), BF16),
            pltpu.VMEM((B, SQ, 2 * D), BF16),
            pltpu.SemaphoreType.DMA((2,)),
            pltpu.SemaphoreType.DMA((2,)),
            pltpu.SemaphoreType.DMA((2,)),
            pltpu.SemaphoreType.DMA((2, NBG)),
            pltpu.SemaphoreType.DMA((2, NPP)),
            pltpu.SemaphoreType.DMA(()),
        ],
        compiler_params=pltpu.CompilerParams(vmem_limit_bytes=120 * 1024 * 1024),
        name="concat_cached_attention",
    )(
        A_x, dims_major(A_k_cache), dims_major(A_v_cache), A_wq, A_wo,
        B_x, dims_major(B_k_cache), dims_major(B_v_cache), B_wq, B_wo,
    )
```
